```python
import os as _os
_os.environ.setdefault("JAX_PLATFORMS", "cpu")
import jax
import jax.numpy as jnp

def _softmax(x, axis=-1):
    return jax.nn.softmax(x, axis=axis)
def _gelu(x):
    return jax.nn.gelu(x, approximate=True)
def _silu(x):
    return jax.nn.silu(x)
def _sigmoid(x):
    return jax.nn.sigmoid(x)
def _layernorm(x, axis=-1, eps=1e-5):
    m = jnp.mean(x, axis=axis, keepdims=True)
    v = jnp.var(x, axis=axis, keepdims=True)
    return (x - m) / jnp.sqrt(v + eps)
def _scatter_add(tgt, idx, src, axis=0):
    return tgt.at[idx].add(src)
def _segment_sum(src, seg, n):
    return jax.ops.segment_sum(src, seg, n)
class _Rng:
    def __init__(self, key):
        self._k = key
    def _next(self):
        self._k, sub = jax.random.split(self._k)
        return sub
    def normal(self, shape):
        return jax.random.normal(self._next(), shape, dtype=jnp.bfloat16)
    def randint(self, lo, hi, shape):
        return jax.random.randint(self._next(), shape, lo, hi, dtype=jnp.int32)
    def uniform(self, shape, lo=0.0, hi=1.0):
        return jax.random.uniform(self._next(), shape, jnp.bfloat16, lo, hi)
    def permutation(self, n):
        return jax.random.permutation(self._next(), n)


kernel_name = 'interleave_layers__linear_kernel_hedgehog__sliding_block__prompt'

def setup_inputs():
    _rng = _Rng(jax.random.key(int.from_bytes(__import__("os").urandom(4), "little")))
    _w = (lambda a: (lambda t: t.astype(jnp.bfloat16) if jnp.issubdtype(t.dtype, jnp.floating) else t)(jnp.asarray(a)))
    def _A_setup():
        B, S, D, H = 1, 2048, 448, 16
        Dh = D // H
        return {
            "x": _w((lambda *s: _rng.normal(s) * 0.05)(B, S, D)),
            "wqkv": _w((lambda *s: _rng.normal(s) * 0.4)(D, 3 * D)),
            "w_phi": _w((lambda *s: _rng.normal(s) * 0.4)(H, Dh, Dh) * (Dh ** -0.5)),
            "wo": _w((lambda *s: _rng.normal(s) * 0.05)(D, D)),
        }
    _A_in = _A_setup()

    def _B_setup():
        B, S, D = 1, 2048, 448
        return {
            "x": _w((lambda *s: _rng.normal(s) * 0.05)(B, S, D)),
            "wqkv": _w((lambda *s: _rng.normal(s) * 0.1)(D, 3 * D)),
            "wo": _w((lambda *s: _rng.normal(s) * 0.1)(D, D)),
        }
    _B_in = _B_setup()

    return {
        "A_x": _A_in["x"],
        "A_wqkv": _A_in["wqkv"],
        "A_w_phi": _A_in["w_phi"],
        "A_wo": _A_in["wo"],
        "B_x": _B_in["x"],
        "B_wqkv": _B_in["wqkv"],
        "B_wo": _B_in["wo"],
    }

def reference(A_x, A_wqkv, A_w_phi, A_wo, B_x, B_wqkv, B_wo):
    def _A_ref(x, wqkv, w_phi, wo):
        B, S, D = x.shape
        H = 16; Dh = D // H
        qkv = (lambda x, *d: x.transpose(*d))((x @ wqkv).reshape(B, S, 3, H, Dh), 2, 0, 3, 1, 4)
        q, k, v = qkv[0], qkv[1], qkv[2]
        pq = jnp.einsum("bhsd,hdf->bhsf", q, w_phi)
        pk = jnp.einsum("bhsd,hdf->bhsf", k, w_phi)
        phi_q = jnp.concatenate([_softmax(pq, axis=-1), _softmax(-pq, axis=-1)], axis=-1)
        phi_k = jnp.concatenate([_softmax(pk, axis=-1), _softmax(-pk, axis=-1)], axis=-1)
        kv = jnp.einsum("bhsf,bhsd->bhfd", phi_k, v)
        z  = jnp.einsum("bhsf->bhf", phi_k)
        num = jnp.einsum("bhqf,bhfd->bhqd", phi_q, kv)
        den = jnp.einsum("bhqf,bhf->bhq", phi_q, z)[..., None] + 1e-6
        o = num / den
        return (lambda x, *d: x.transpose(*d))(o, 0, 2, 1, 3).reshape(B, S, D) @ wo

    def _B_ref(x, wqkv, wo):
        B, S, D = x.shape
        H = 16; Dh = D // H; W = 256
        qkv = (lambda x, *d: x.transpose(*d))((x @ wqkv).reshape(B, S, 3, H, Dh), 2, 0, 3, 1, 4)
        q, k, v = qkv[0], qkv[1], qkv[2]
        scores = jnp.einsum("bhqd,bhkd->bhqk", q, k) * (Dh ** -0.5)
        idx = jnp.arange(S)
        mask = (idx[:, None] - idx[None, :] >= 0) & (idx[:, None] - idx[None, :] < W)
        scores = jnp.where(mask[None, None], scores, -1e9)
        p = _softmax(scores, axis=-1)
        o = jnp.einsum("bhqk,bhkd->bhqd", p, v)
        return (lambda x, *d: x.transpose(*d))(o, 0, 2, 1, 3).reshape(B, S, D) @ wo

    x = A_x
    x = x + _A_ref(_layernorm(x, axis=-1), A_wqkv, A_w_phi, A_wo)
    x = x + _B_ref(_layernorm(x, axis=-1), B_wqkv, B_wo)
    x = x + _A_ref(_layernorm(x, axis=-1), A_wqkv, A_w_phi, A_wo)
    x = x + _B_ref(_layernorm(x, axis=-1), B_wqkv, B_wo)
    return x
```

```python
import math

import jax
import jax.numpy as jnp
import jax.experimental.pallas as pl
import jax.experimental.pallas.tpu as pltpu

S, D, H, DH, WIN = 2048, 448, 16, 28, 256
NB = S // 128
IN_CUTS = (0, 2, 8, 16)
OUT_CUTS = (0, 8, 13, 15, 16)
HD = D // 2
AQ, AK, AV, AO, BQ, BK, BV, BO = range(8)
SOURCE = (0, 0, 0, 2, 1, 1, 1, 3)
FAST = (0, 1)
PREP = 20
QLEAD = 8
GAP = (0, 0, 1, 0, 1, 0)
DL = (2, -1, -1, -1)
LOG2E = math.log2(math.e)
F32, BF16, U32, I32 = jnp.float32, jnp.bfloat16, jnp.uint32, jnp.int32
NT_DIMS = (((1,), (1,)), ((), ()))


def _iota(shape, dim):
    return jax.lax.broadcasted_iota(I32, shape, dim)


def _dot(a, b):
    return jnp.dot(a, b, preferred_element_type=F32)


def _words(x):
    return pltpu.bitcast(x.astype(BF16), I32)


def _zip(lo, hi):
    return pltpu.bitcast(pltpu.pack_elementwise([lo, hi], packed_dtype=BF16), I32)


def _strassen_left(a11, a12, a21, a22):
    return [a11 + a22, a22, a11 + a12, a12 - a22, a21 + a22, a11, a21 - a11]


def _strassen_right(b11, b12, b21, b22):
    return [b11 + b22, b21 - b11, b22, b21 + b22, b11, b12 - b22, b11 + b12]


STRASSEN_OUT = (
    (((0, 0), 1), ((1, 1), 1)), (((0, 0), 1), ((0, 1), 1)),
    (((0, 0), -1), ((1, 0), 1)), (((0, 0), 1),),
    (((0, 1), 1), ((1, 1), -1)), (((1, 0), 1), ((1, 1), 1)), (((1, 1), 1),))
STRASSEN_ROUNDS = (
    ((0, 0), (3, 0)), ((1, 0), (4, 0)), ((2, 0), (5, 0)), ((6, 0), (0, 1)),
    ((1, 1), (4, 1)), ((2, 1), (5, 1)), ((3, 1), (6, 1)), ())


def _recip(x):
    r = pl.reciprocal(x, approx=True)
    return r * (2.0 - x * r)


def _bf(w):
    return pltpu.bitcast(w, BF16)


def _div28(v):
    return (v * 2341) >> 16


def _pair_reduce(op, x):
    r = x[0:8]
    for i in range(1, 7):
        r = op(r, x[8 * i:8 * i + 8])
    r = op(r, pltpu.roll(r, 4, 0))
    return op(r, pltpu.roll(r, 2, 0))


def _feature_map(p):
    rep = lambda r: jnp.concatenate([r] * 7, axis=0)
    ep = jnp.exp2(p - rep(_pair_reduce(jnp.maximum, p)))
    en = jnp.exp2(rep(_pair_reduce(jnp.minimum, p)) - p)
    fp = ep * rep(_recip(_pair_reduce(jnp.add, ep)))
    fn = en * rep(_recip(_pair_reduce(jnp.add, en)))
    return _zip(fp, fn)


def _pair_scale(num, mixed):
    r = _recip(mixed)
    sw = pltpu.roll(r, 4, 0)
    lo = _iota(r.shape, 0) < 4
    ra, rb = jnp.where(lo, r, sw), jnp.where(lo, sw, r)
    return num * jnp.concatenate([ra, ra, ra, r, rb, rb, rb], axis=0)


def _kernel(x_hbm, awqkv_hbm, aphi_hbm, awo_hbm, bwqkv_hbm, bwo_hbm, o_hbm,
            xio, rawa, rawb, rawoa, rawob, praw, pf32, wst, wf, wt, ws,
            rhs, part, fk, va, fq, att, pbuf, xt, kv, kvm, qr, kn, vp, qmask, pmask, zero,
            wsems, xsems, osems):
    def pieces(src, dst, cuts, sems):
        cols = [pl.ds(128 * a, 128 * (b - a)) for a, b in zip(cuts, cuts[1:])]
        return [pltpu.make_async_copy(src.at[:, c], dst.at[:, c], sems.at[i])
                for i, c in enumerate(cols)]

    x_copies = pieces(x_hbm, xio, IN_CUTS, xsems)
    o_copies = pieces(xio, o_hbm, OUT_CUTS, osems)
    w_pairs = [(awqkv_hbm.at[:, c], rawa.at[:, c])
               for c in (pl.ds(896, D), pl.ds(384, 512), pl.ds(0, 384))]
    w_pairs += [(awo_hbm, rawoa), (bwqkv_hbm, rawb), (bwo_hbm, rawob)]
    w_copies = [pltpu.make_async_copy(a, b, wsems.at[i])
                for i, (a, b) in enumerate(w_pairs)]
    phi_copy = pltpu.make_async_copy(aphi_hbm, praw, wsems.at[6])
    for cp in (x_copies[0], phi_copy, w_copies[0], w_copies[1]):
        cp.start()

    for buf in (rhs, part, fk, va, fq, att, pbuf, xt, qr, kn, vp, qmask, pmask, zero):
        buf[(0,) * (len(buf.shape) - 2) + (pl.ds(0, 8), pl.ds(0, 64))] = jnp.zeros(
            (8, 64), buf.dtype)

    zero[:, 64:128] = jnp.zeros((8, 64), I32)

    row, lane = _iota((64, 128), 0), _iota((64, 128), 1)
    for t in range(4):
        head = _div28(row) + t
        qmask[t] = (jnp.where((lane >> 5) == (head & 3), 0xFFFF, 0)
                    | jnp.where((lane >> 5) == ((head + 2) & 3), -65536, 0))
    key, qry = 2 * row[0:16], lane[0:16] & 31
    newer = jnp.where(key <= qry, 0xFFFF, 0) | jnp.where(key + 1 <= qry, -65536, 0)
    pmask[0] = ~newer
    pmask[1] = newer
    wst[...] = jnp.zeros(wst.shape, F32)
    pf32[...] = jnp.zeros(pf32.shape, F32)
    phi_copy.wait()
    pf32[:, 0:DH] = praw[...].astype(F32)
    for h in range(H):
        wst[h // 4, DH * (h % 4):DH * (h % 4 + 1)] = pf32[pl.ds(h, DH, stride=H), :]
    crow, ccol = _iota((112, 128), 0), _iota((112, 128), 1)
    hi = crow >= 56
    expand = (((crow - jnp.where(hi, 56, 0)) >> 1) == ccol).astype(F32).astype(BF16)
    same = (jnp.where(hi, 2, 0) + (crow & 1)) == _div28(ccol)
    bdt = []
    for g in range(4):
        full = jax.lax.dot_general(expand, wst[g].astype(BF16), NT_DIMS,
                                   preferred_element_type=F32)
        bdt.append(jnp.where(same, full, 0.0)[:, 0:112].astype(BF16))

    xna, xnb, oa, ob = range(4)
    live = {}

    due = [[] for _ in range(4)]

    def pin(x, delay=0):
        if delay < 0:
            return x
        x = x if x.dtype == I32 else pltpu.bitcast(x, I32)
        due[delay] += [x[i:i + 8] for i in range(0, x.shape[0], 8)]
        return x

    def after_pinned(words):
        vals = due.pop(0)
        due.append([])
        if not vals:
            return words
        nothing = zero[...]
        for v in vals:
            nothing = nothing & v
        head = words[0:8, 0:128] | nothing
        if words.shape[1] > 128:
            head = jnp.concatenate([head, words[0:8, 128:]], axis=1)
        return jnp.concatenate([head, words[8:]], axis=0)

    def feed(dst, rows):
        def plain(c, g):
            for i in range(56 * g, 56 * g + 56, 8):
                j = i + 112 * (g // 2)
                rhs[dst, c // 2, 2 * (c % 2) + g // 2, i % 112:i % 112 + 8] = pin(
                    _zip(rows(c, j), rows(c, j + 112)), DL[0])

        def stage(c, g):
            if c % 2:
                return
            for i in range(32 * g, min(32 * g + 32, 112), 8):
                lo, hi = [_strassen_right(*[rows(b, kh + i + off) for kh in (0, HD)
                                            for b in (c, c + 1)]) for off in (0, 112)]
                for r in range(7):
                    rhs[dst, c // 2, r, i:i + 8] = pin(_zip(lo[r], hi[r]), DL[0])
        return stage if dst in FAST else plain

    def proj(w, src, post):
        def plain(c, g):
            right = [rhs[src, c // 2, 2 * (c % 2) + kh] for kh in range(2)]
            post(c, g, _dot(_bf(after_pinned(wf[pl.ds(w * HD + 56 * g, 56)])),
                            _bf(jnp.concatenate(right, axis=0))))

        def stage(c, g):
            cur = {}
            for r, h in STRASSEN_ROUNDS[4 * (c % 2) + g]:
                left = ws[w, r, pl.ds(56 * h, 56)]
                left = left if cur else after_pinned(left)
                m = _dot(_bf(left), _bf(rhs[src, c // 2, r]))
                for (b, half), sign in STRASSEN_OUT[r]:
                    key = (w, b, 2 * h + half)
                    n = live.get(key, 0)
                    if n:
                        acc = cur[key] if key in cur else part[key]
                        cur[key] = acc + m if sign > 0 else acc - m
                    else:
                        cur[key] = m
                    live[key] = (n + 1) % (4 if b == half else 2)
            for key, acc in cur.items():
                if live[key]:
                    part[key] = acc
                else:
                    post(c - c % 2 + key[1], key[2], acc)
        return stage if src in FAST else plain

    def a_k(c, g, pk):
        for e in range(2):
            fk[c % 4, 2 * g + e] = pin(_feature_map(pk[56 * e:56 * e + 56]), DL[1])

    def a_v(c, g, v):
        for e in range(2):
            va[c % 4, 2 * g + e] = _words(jnp.concatenate(
                [v[56 * e:56 * e + 56], jnp.ones((8, 128), F32)], axis=0))

    def a_kv(c, g):
        if g % 2 == 0:
            return
        for gg in (g - 1, g):
            for e in range(2):
                p = 2 * gg + e
                upd = jax.lax.dot_general(_bf(va[c % 4, p]), _bf(fk[c % 4, p]),
                                          NT_DIMS, preferred_element_type=F32)
                if c > 0:
                    upd = kv[p] + upd
                if c < NB - 1:
                    kv[p] = upd
                else:
                    r, col = _iota((64, 112), 0), _iota((64, 112), 1)
                    second = ((r >= DH) & (r < 56)) | (r >= 60)
                    kvm[p] = _words(jnp.where(second == ((col & 2) == 2), upd, 0.0))

    def a_q(c, g, pq):
        for e in range(2):
            fq[c, 2 * g + e] = pin(_feature_map(pq[56 * e:56 * e + 56]), DL[2])

    def a_num(c, g):
        if g % 2 == 0:
            return
        for p in range(2 * g - 2, 2 * g + 2):
            nd = _dot(_bf(kvm[p]), _bf(fq[c, p]))
            att[0, c % 4, pl.ds(56 * p, 56)] = _pair_scale(nd[0:56], nd[56:64] + 1e-6)

    def residual(c, g, y):
        xt[c, pl.ds(112 * g, 112)] += y

    def stats(dst):
        def stage(c, g):
            if c % 2:
                return
            b = c + g // 2
            if g % 2 == 0:
                m = jnp.sum(xt[b], axis=0, keepdims=True) * (1.0 / D)
                live[dst, b] = last = jnp.broadcast_to(m, (8, 128))
            else:
                m = live[dst, b]
                d = xt[b] - m[0:1]
                v = jnp.sum(d * d, axis=0, keepdims=True) * (1.0 / D)
                r = jnp.broadcast_to(jax.lax.rsqrt(v + 1e-5), (8, 128))
                last = m * r
                live[dst, b] = (r, last)
            pin(last, DL[0])
        return stage

    def norm(dst):
        return feed(dst, lambda b, i: (xt[b, i:i + 8] * live[dst, b][0]
                                       - live[dst, b][1]))

    def b_k(c, g, k):
        k = jnp.concatenate([_zip(k[0:56], k[56:112]), jnp.zeros((8, 128), I32)], axis=0)
        k = pltpu.bitcast(_bf(k).T, I32)
        kn[g, 0, pl.ds(c * 32, 32)] = _words(pltpu.bitcast(k << 16, F32))
        kn[g, 1, pl.ds(c * 32, 32)] = _words(pltpu.bitcast(k & -65536, F32))

    def b_q(c, g, q):
        q = q * (DH ** -0.5 * LOG2E)
        lo = _iota((8, 128), 0) < 4
        r1 = pltpu.roll(q[24:56], 32, 1)
        r2 = pltpu.roll(q[56:88], 64, 1)
        r3 = pltpu.roll(q[80:112], 96, 1)
        qr[c, g] = _zip(
            jnp.concatenate(
                [q[0:24], jnp.where(lo, q[24:32], r1[0:8]), r1[8:32]], axis=0),
            jnp.concatenate(
                [r2[0:24], jnp.where(lo, r2[24:32], r3[0:8]), r3[8:32]], axis=0))

    def b_v(c, g, v):
        lo = _iota((8, 128), 0) < 4
        for e in range(2):
            ve = v[56 * e:56 * e + 56]
            vp[c, 4 * g + 2 * e] = _words(jnp.concatenate(
                [ve[0:24], jnp.where(lo, ve[24:32], 1.0)], axis=0))
            vp[c, 4 * g + 2 * e + 1] = _words(jnp.concatenate(
                [jnp.where(lo, 1.0, ve[24:32]), ve[32:56]], axis=0))

    def scores(blk, g):
        q = qr[blk, g]
        out = [None] * 4
        for t in (3, 2, 1, 0) if g % 2 else (0, 1, 2, 3):
            qt = _bf(jnp.concatenate(
                [q & qmask[t, 0:56], jnp.zeros((8, 128), I32)], axis=0))
            end = blk * 128 + 32 * t + 32
            start = max(end - 288, 0)
            keys = [kn[g, i, start // 4:end // 4] for i in range(2)]
            keys = jnp.concatenate(keys, axis=0)
            out[t] = _dot(_bf(keys if t else after_pinned(keys)), qt)
        return out

    def b_qk(c, g):
        key, qry = 2 * _iota((16, 128), 0), _iota((16, 128), 1) & 31
        for t, s in enumerate(scores(c, g)):
            n = s.shape[0] // 2
            halves = []
            for i in range(2):
                h = s[i * n:i * n + n]
                edge = jnp.where(key + i <= qry, h[n - 16:],
                                 h[0:16] if n == 144 else -1e9 * LOG2E)
                halves.append(jnp.concatenate(
                    [h[max(n - 128, 0):n - 16], edge], axis=0) if n > 16 else edge)
            m = jnp.max(jnp.concatenate(halves, axis=0), axis=0, keepdims=True)
            live["s", g, t] = (halves, m)

    def b_exp(t):
        def stage(c, g):
            halves, m = live.pop(("s", g, t))
            pbuf[g, t, 128 - halves[0].shape[0]:] = pin(
                _zip(*[jnp.exp2(h - m) for h in halves]), DL[3])
        return stage

    def b_pv(i):
        def pick(cond, a, b):
            if a is None and b is None:
                return None
            return jnp.where(cond, 0 if a is None else a, 0 if b is None else b)

        def stage(c, g):
            if c - 2 + i < 0:
                return
            ln = _iota((16, 128), 1)
            odd, upper = (ln & 32) != 0, (ln & 64) != 0
            heads = [[] for _ in range(4)]
            for u in range(4):
                pc = []
                for t in range(4):
                    k = 4 * i + u - t
                    if k in (0, 8):
                        pc.append(pbuf[g, t, 112:128] & pmask[k // 8])
                    else:
                        pc.append(pbuf[g, t, 16 * k - 16:16 * k] if 0 < k < 8 else None)
                y = [pick(odd, pc[(k + 1) % 4], pc[k]) for k in range(4)]
                for j in range(4):
                    heads[j].append(pick(upper, y[(2 - j) % 4], y[(-j) % 4]))
            acc = live.get(("o", c, g))
            res = [_dot(_bf(vp[c - 2 + i, 4 * g + j]),
                        _bf(jnp.concatenate(heads[j], axis=0))) for j in range(4)]
            live["o", c, g] = res if acc is None else [a + o for a, o in zip(acc, res)]
        return stage

    def b_fin(c, g):
        res = [o if j == 0 else pltpu.roll(o, 128 - 32 * j, 1)
               for j, o in enumerate(live.pop(("o", c, g)))]
        lo = _iota((8, 128), 0) < 4
        outs = []
        for e in range(2):
            u, w = res[2 * e], res[2 * e + 1]
            num = jnp.concatenate(
                [u[0:24], jnp.where(lo, u[24:32], w[0:8]), w[8:32]], axis=0)
            den = pltpu.roll(jnp.where(lo, w[0:8], u[24:32]), 4, 0)
            outs.append(_pair_scale(num, den))
        att[1, c % 4, pl.ds(112 * g, 112)] = jnp.concatenate(outs, axis=0)

    def b_out(c, g, y):
        rows = pl.ds(112 * g, 112)
        xio[rows, 128 * c:128 * c + 128] = (xt[c, rows] + y).astype(BF16)
        if g == 3 and c + 1 in OUT_CUTS:
            o_copies[OUT_CUTS.index(c + 1) - 1].start()

    def load_x(c, g):
        if g == 0:
            if c in IN_CUTS[2:]:
                x_copies[IN_CUTS.index(c)].wait()
            xt[c] = xio[:, 128 * c:128 * c + 128].astype(F32)

    def transpose(w, src, i):
        n = min(128, src.shape[1] - i)
        rows = pl.ds((w * D + i) // 2, n // 2)
        a = src[:, i:i + n].astype(F32)
        a = [_zip(a[j:j + 112], a[j + 112:j + HD]) for j in (0, HD)]
        if SOURCE[w] in FAST:
            for kh in range(2):
                wt[kh, rows] = _words(_bf(a[kh]).T)
        else:
            wf[rows] = _words(_bf(jnp.concatenate(a, axis=0)).T)

    def factors(w, h):
        if SOURCE[w] not in FAST:
            for g in (2 * h, 2 * h + 1) if w in (AQ, AK) else ():
                rows = pl.ds(w * HD + 56 * g, 56)
                wf[rows] = _words(_dot(bdt[g], _bf(wf[rows])) * LOG2E)
            return
        quad = []
        for g in (2 * h, 2 * h + 1):
            for kh in range(2):
                a = _bf(wt[kh, pl.ds(w * HD + 56 * g, 56)])
                if w in (AQ, AK):
                    quad.append(_dot(bdt[g], a) * LOG2E)
                else:
                    quad.append(a.astype(F32))
        for r, a in enumerate(_strassen_left(*quad)):
            ws[w, r, pl.ds(56 * h, 56)] = _words(a)

    late = []
    for cp, w, src, n in zip(w_copies[2:], (AQ, AO, BQ, BO),
                             (rawa, rawoa, rawb, rawob), (384, D, 3 * D, D)):
        late += [(cp.wait,)] + [(transpose, w, src, i) for i in range(0, n, 128)]
        late += [(factors, w + j, h) for j in range(max(n // D, 1)) for h in range(2)]

    def prep(c, g):
        for step in late[4 * c + g:4 * c + g + 1]:
            step[0](*step[1:])

    x_copies[0].wait()
    x_copies[1].start()
    for c in range(2):
        load_x(c, 0)
    for stage in (stats(xna), norm(xna)):
        for g in range(4):
            stage(0, g)
    w_copies[0].wait()
    for i in range(896, 3 * D, 128):
        transpose(AQ, rawa, i)
    for h in range(2):
        factors(AV, h)
    w_copies[1].wait()
    x_copies[1].wait()
    for cp in x_copies[2:] + w_copies[2:]:
        cp.start()
    for i in range(384, 896, 128):
        transpose(AQ, rawa, i)
    for c in (2, 3):
        load_x(c, 0)
    for g in range(4):
        proj(AV, xna, a_v)(0, g)
        stats(xna)(2, g)
    for h in range(2):
        factors(AK, h)

    U = 4 * NB
    plan = [(load_x, -16), (prep, PREP), (stats(xna), -12), (norm(xna), -8),
            (proj(AV, xna, a_v), -4), (proj(AK, xna, a_k), 0), (a_kv, 4)]
    t0 = U + 3
    for last in (False, True):
        la, lb = (8 if oa in FAST else 2), (8 if ob in FAST else 2)
        t1 = t0 + la + 4 + GAP[0]
        t2 = t1 + 15 + GAP[1]
        t3 = t2 + 6 + GAP[2]
        t4 = t3 + 2 + GAP[3]
        t5 = t4 + lb + 4 + GAP[4]
        t6 = t5 + 15 + GAP[5]
        plan += [
            (b_qk, t3), (stats(xnb), t1 + 7), (norm(xnb), t1 + 11),
            (proj(AO, oa, residual), t1), (b_pv(0), t4), (b_exp(0), t3 + 1),
            (proj(BO, ob, b_out if last else residual), t5), (b_pv(2), t4), (b_exp(1), t3 + 1),
            (proj(AQ, xna, a_q), t0 - QLEAD),
            (b_pv(1), t4),
            (feed(oa, lambda b, i: att[0, b % 4, i:i + 8]), t0 + la),
            (feed(ob, lambda b, i: att[1, b % 4, i:i + 8]), t4 + lb),
            (proj(BK, xnb, b_k), t2), (b_fin, t4), (a_num, t0), (b_exp(2), t3 + 1),
            (proj(BQ, xnb, b_q), t2 + 1), (b_exp(3), t3 + 1),
            (proj(BV, xnb, b_v), t2 + 2)]
        if not last:
            plan += [(proj(AK, xna, a_k), t6), (stats(xna), t5 + 7),
                     (norm(xna), t5 + 11), (proj(AV, xna, a_v), t6 + 1),
                     (a_kv, t6 + 5)]
        t0 = t6 + U + 4
    for u in range(max(t for _, t in plan) + U):
        for stage, t in plan:
            if 0 <= u - t < U:
                stage(*divmod(u - t, 4))

    for cp in o_copies:
        cp.wait()


@jax.jit
def pallas_interleave_layers__linear_kernel_hedgehog__sliding_block__prompt_kernel(
    A_x: jax.Array,
    A_wqkv: jax.Array,
    A_w_phi: jax.Array,
    A_wo: jax.Array,
    B_x: jax.Array,
    B_wqkv: jax.Array,
    B_wo: jax.Array,
):
    del B_x
    hbm = pl.BlockSpec(memory_space=pltpu.MemorySpace.HBM)
    out = pl.pallas_call(
        _kernel,
        out_shape=jax.ShapeDtypeStruct((D, S), A_x.dtype),
        in_specs=[hbm] * 6,
        out_specs=hbm,
        scratch_shapes=[
            pltpu.VMEM((D, S), BF16),
            pltpu.VMEM((D, 3 * D), BF16),
            pltpu.VMEM((D, 3 * D), BF16),
            pltpu.VMEM((D, D), BF16),
            pltpu.VMEM((D, D), BF16),
            pltpu.VMEM((D, DH), BF16),
            pltpu.VMEM((D, 128), F32),
            pltpu.VMEM((4, 128, 128), F32),
            pltpu.VMEM((8 * HD, D), I32),
            pltpu.VMEM((2, 8 * HD, HD), I32),
            pltpu.VMEM((8, 7, HD // 2, HD), I32),
            pltpu.VMEM((4, NB // 2, 7, HD // 2, 128), I32),
            pltpu.VMEM((8, 2, 4, 112, 128), F32),
            pltpu.VMEM((4, 8, 56, 128), I32),
            pltpu.VMEM((4, 8, 32, 128), I32),
            pltpu.VMEM((NB, 8, 56, 128), I32),
            pltpu.VMEM((2, 4, D, 128), F32),
            pltpu.VMEM((4, 4, 128, 128), I32),
            pltpu.VMEM((NB, D, 128), F32),
            pltpu.VMEM((8, 64, 112), F32),
            pltpu.VMEM((8, 32, 112), I32),
            pltpu.VMEM((NB, 4, 56, 128), I32),
            pltpu.VMEM((4, 2, S // 4, 128), I32),
            pltpu.VMEM((NB, H, 16, 128), I32),
            pltpu.VMEM((4, 64, 128), I32),
            pltpu.VMEM((2, 16, 128), I32),
            pltpu.VMEM((8, 128), I32),
            pltpu.SemaphoreType.DMA((7,)),
            pltpu.SemaphoreType.DMA((len(IN_CUTS) - 1,)),
            pltpu.SemaphoreType.DMA((len(OUT_CUTS) - 1,)),
        ],
        compiler_params=pltpu.CompilerParams(vmem_limit_bytes=96 * 1024 * 1024),
    )(A_x.reshape(S, D).T, A_wqkv, A_w_phi.transpose(1, 0, 2).reshape(D, DH),
      A_wo, B_wqkv, B_wo)
    return out.T.reshape(A_x.shape)
```

```python
import math

import jax
import jax.numpy as jnp
import jax.experimental.pallas as pl
import jax.experimental.pallas.tpu as pltpu

S, D, H, DH = 2048, 448, 16, 28
NB = S // 128
IN_CUTS = (0, 2, 8, 16)
OUT_CUTS = (0, 8, 13, 15, 16)
HD = D // 2
AQ, AK, AV, BQ, BK, BV = range(6)
GAP = ((0, 4, 2, 0, 1, 0, 0, 4, 0, 0, 2, 1, 1), (0, 2, 0, 0, 0, 2, 2, 4, 0, 0, 2, 2, 2))
ORDER = ('Sn01OeWQKHNVlmoFG2Z', 'OnNFel0VWQKS12')
SKEW = 24
ALIGN = (2, 9)
RESET = (36,)
NORM_DUE, STATS_DUE, PREP_DUE, KEYS_DUE = 2, 4, 3, 3
LOG2E = math.log2(math.e)
F32, BF16, I32 = jnp.float32, jnp.bfloat16, jnp.int32
NT_DIMS = (((1,), (1,)), ((), ()))


def _iota(shape, dim):
    return jax.lax.broadcasted_iota(I32, shape, dim)


def _dot(a, b):
    return jnp.dot(a, b, preferred_element_type=F32)


def _words(x):
    return pltpu.bitcast(x.astype(BF16), I32)


def _zip(lo, hi):
    return pltpu.bitcast(pltpu.pack_elementwise([lo, hi], packed_dtype=BF16), I32)


def _unzip(w):
    return pltpu.bitcast(w << 16, F32), pltpu.bitcast(w & -65536, F32)


def _strassen_left(a11, a12, a21, a22):
    return [a11 + a22, a22, a11 + a12, a12 - a22, a21 + a22, a11, a21 - a11]


def _strassen_right(b11, b12, b21, b22):
    return [b11 + b22, b21 - b11, b22, b21 + b22, b11, b12 - b22, b11 + b12]


STRASSEN_OUT = (
    (((0, 0), 1), ((1, 1), 1)), (((0, 0), 1), ((0, 1), 1)),
    (((0, 0), -1), ((1, 0), 1)), (((0, 0), 1),),
    (((0, 1), 1), ((1, 1), -1)), (((1, 0), 1), ((1, 1), 1)), (((1, 1), 1),))
STRASSEN_ROUNDS = (
    ((0, 0), (3, 0)), ((1, 0), (4, 0)), ((2, 0), (5, 0)), ((6, 0), (0, 1)),
    ((1, 1), (4, 1)), ((2, 1), (5, 1)), ((3, 1), (6, 1)), ())


def _recip(x):
    r = pl.reciprocal(x, approx=True)
    return r * (2.0 - x * r)


def _bf(w):
    return pltpu.bitcast(w, BF16)


def _div28(v):
    return (v * 2341) >> 16


def _pair_reduce(op, x):
    r = x[0:8]
    for i in range(1, 7):
        r = op(r, x[8 * i:8 * i + 8])
    r = op(r, pltpu.roll(r, 4, 0))
    return op(r, pltpu.roll(r, 2, 0))


def _feature_map(p):
    rep = lambda r: jnp.concatenate([r] * 7, axis=0)
    ep = jnp.exp2(p - rep(_pair_reduce(jnp.maximum, p)))
    en = jnp.exp2(rep(_pair_reduce(jnp.minimum, p)) - p)
    fp = ep * rep(_recip(_pair_reduce(jnp.add, ep)))
    fn = en * rep(_recip(_pair_reduce(jnp.add, en)))
    return _zip(fp, fn)


def _pair_scale(num, mixed):
    r = _recip(mixed)
    sw = pltpu.roll(r, 4, 0)
    lo = _iota(r.shape, 0) < 4
    ra, rb = jnp.where(lo, r, sw), jnp.where(lo, sw, r)
    return num * jnp.concatenate([ra, ra, ra, r, rb, rb, rb], axis=0)


def _kernel(x_hbm, awqkv_hbm, aphi_hbm, awo_hbm, bwqkv_hbm, bwo_hbm, o_hbm,
            xio, rawa, rawb, rawoa, rawob, praw, pf32, wst, wo, wt, ws,
            rhs, part, fk, va, fq, att, pbuf, xt, kv, kvm, qr, kn, vp, qmask, pmask, zero,
            wsems, xsems, osems):
    def pieces(src, dst, cuts, sems):
        cols = [pl.ds(128 * a, 128 * (b - a)) for a, b in zip(cuts, cuts[1:])]
        return [pltpu.make_async_copy(src.at[:, c], dst.at[:, c], sems.at[i])
                for i, c in enumerate(cols)]

    x_copies = pieces(x_hbm, xio, IN_CUTS, xsems)
    o_copies = pieces(xio, o_hbm, OUT_CUTS, osems)
    w_pairs = [(awqkv_hbm.at[:, c], rawa.at[:, c])
               for c in (pl.ds(896, D), pl.ds(384, 512), pl.ds(0, 384))]
    w_pairs += [(awo_hbm, rawoa), (bwqkv_hbm, rawb), (bwo_hbm, rawob)]
    w_copies = [pltpu.make_async_copy(a, b, wsems.at[i])
                for i, (a, b) in enumerate(w_pairs)]
    phi_copy = pltpu.make_async_copy(aphi_hbm, praw, wsems.at[6])
    for cp in (x_copies[0], phi_copy, w_copies[0], w_copies[1], x_copies[1]):
        cp.start()

    for buf in (rhs, part, fk, va, fq, att, pbuf, xt, qr, kn, vp, qmask, pmask, zero):
        buf[(0,) * (len(buf.shape) - 2) + (pl.ds(0, 8), pl.ds(0, 64))] = jnp.zeros(
            (8, 64), buf.dtype)

    zero[:, 64:128] = jnp.zeros((8, 64), I32)

    row, lane = _iota((64, 128), 0), _iota((64, 128), 1)
    for t in range(4):
        head = _div28(row) + t
        qmask[t] = (jnp.where((lane >> 5) == (head & 3), 0xFFFF, 0)
                    | jnp.where((lane >> 5) == ((head + 2) & 3), -65536, 0))
    key, qry = 2 * row[0:16], lane[0:16] & 31
    newer = jnp.where(key <= qry, 0xFFFF, 0) | jnp.where(key + 1 <= qry, -65536, 0)
    pmask[0] = ~newer
    pmask[1] = newer
    wst[...] = jnp.zeros(wst.shape, F32)
    pf32[...] = jnp.zeros(pf32.shape, F32)
    bdt = []

    def load_phi():
        phi_copy.wait()
        pf32[0:D, 0:DH] = praw[...].astype(F32)
        for h in range(H):
            wst[h // 4, DH * (h % 4):DH * (h % 4 + 1)] = pf32[pl.ds(h, DH, stride=H), :]
        crow, ccol = _iota((112, 128), 0), _iota((112, 128), 1)
        quarter = _div28(crow)
        expand = ((crow - DH * quarter) == ccol).astype(F32).astype(BF16)
        same = (2 * (quarter & 1) + (quarter >> 1)) == _div28(ccol)
        for g in range(4):
            full = jax.lax.dot_general(expand, wst[g].astype(BF16), NT_DIMS,
                                       preferred_element_type=F32)
            bdt.append(jnp.where(same, full, 0.0)[:, 0:112].astype(BF16))

    xna, xnb = range(2)
    live = {}

    stagger = []
    due = [[] for _ in range(6)]

    def pin(x, delay):
        x = x if x.dtype == I32 else pltpu.bitcast(x, I32)
        due[delay] += [x[i:i + 8, j:j + 128] for i in range(0, x.shape[0], 8)
                       for j in range(0, x.shape[1] - 127, 128)]
        return x

    def spread(results, row):
        for i in range(row, row + 4 * SKEW, SKEW):
            v = zero[...]
            for m in results:
                v = v & pltpu.bitcast(m[i:i + 8], I32)
            stagger.append(v)

    def next_round():
        vals = due.pop(0)
        due.append([])
        if not vals and not stagger:
            return _bf
        nothing = zero[...]
        for v in vals:
            nothing = nothing & v

        def gate(words):
            n = words.shape[1]
            wide = jnp.concatenate(
                [nothing | stagger.pop(0) if stagger else nothing
                 for _ in range(pl.cdiv(n, 128))], axis=1)[:, 0:n]
            return _bf(jnp.concatenate([words[0:8] | wide, words[8:]], axis=0))
        return gate

    def out_proj(i, post):
        def stage(c, g):
            left = next_round()(wo[i, pl.ds(56 * g, 56)])
            post(c, g, _dot(left, _bf(att[i, c % 4])))
        return stage

    def proj(w, post):
        def stage(c, g):
            cur, products = {}, []
            for r, h in STRASSEN_ROUNDS[4 * (c % 2) + g]:
                gate = gate if cur else next_round()
                m = _dot(gate(ws[w, r, pl.ds(56 * h, 56)]), _bf(rhs[w // 3, c // 2, r]))
                products.append(m)
                for (b, half), sign in STRASSEN_OUT[r]:
                    key = (w, b, 2 * h + half)
                    terms = live.get(key, 0)
                    if terms:
                        acc = cur[key] if key in cur else part[key]
                        cur[key] = acc + m if sign > 0 else acc - m
                    else:
                        cur[key] = m
                    live[key] = (terms + 1) % (4 if b == half else 2)
            if products and live.pop("spread", False):
                spread(products, 0)
            for key, acc in cur.items():
                if live[key]:
                    part[key] = acc
                else:
                    post(c - c % 2 + key[1], key[2], acc)
        return stage

    def a_k(c, g, pk, first=False):
        for e in range(2):
            f = _feature_map(pk[56 * e:56 * e + 56])
            fk[c % 4, 2 * g + e] = pin(f, KEYS_DUE) if first else f

    def a_v(c, g, v):
        for e in range(2):
            va[c % 4, 2 * g + e] = _words(jnp.concatenate(
                [v[56 * e:56 * e + 56], jnp.ones((8, 128), F32)], axis=0))

    def a_kv(c, g):
        if g % 2 == 0:
            return
        for gg in (g - 1, g):
            for e in range(2):
                p = 2 * gg + e
                upd = jax.lax.dot_general(_bf(va[c % 4, p]), _bf(fk[c % 4, p]),
                                          NT_DIMS, preferred_element_type=F32)
                if c > 0:
                    upd = kv[p] + upd
                if c < NB - 1:
                    kv[p] = upd
                else:
                    r, col = _iota((64, 112), 0), _iota((64, 112), 1)
                    second = ((r >= DH) & (r < 56)) | (r >= 60)
                    kvm[p] = _words(jnp.where(second == ((col & 2) == 2), upd, 0.0))

    def a_q(c, g, pq):
        for e in range(2):
            fq[c, 2 * g + e] = _feature_map(pq[56 * e:56 * e + 56])

    def a_num(c, g):
        if g % 2 == 0:
            return
        for gg in (g - 1, g):
            nds = [_dot(_bf(kvm[p]), _bf(fq[c, p])) for p in (2 * gg, 2 * gg + 1)]
            att[0, c % 4, pl.ds(56 * gg, 56)] = _zip(
                *[_pair_scale(nd[0:56], nd[56:64] + 1e-6) for nd in nds])

    def residual(c, g, y):
        xt[c, pl.ds(112 * g, 112)] += y

    def stats(dst):
        def stage(c, g):
            if c % 2:
                return
            b = c + g // 2
            x = xt[b]
            if g % 2:
                m = live[dst, b]
                x = (x - m[0:1]) * (x - m[0:1])
            mean = jnp.sum(x, axis=0, keepdims=True) * (1.0 / D)
            last = jnp.broadcast_to(mean, (8, 128))
            if g % 2:
                r = jax.lax.rsqrt(last + 1e-5)
                last = m * r
                live[dst, b] = (r, last)
            else:
                live[dst, b] = last
            pin(last, STATS_DUE)
        return stage

    def norm(dst):
        def rows(b, i):
            return xt[b, i:i + 8] * live[dst, b][0] - live[dst, b][1]

        def stage(c, g):
            if c % 2:
                return
            for i in range(32 * g, min(32 * g + 32, 112), 8):
                lo, hi = [_strassen_right(*[rows(b, kh + i + off) for kh in (0, HD)
                                            for b in (c, c + 1)]) for off in (0, 112)]
                for r in range(7):
                    rhs[dst, c // 2, r, i:i + 8] = pin(_zip(lo[r], hi[r]), NORM_DUE)
        return stage

    def b_k(c, g, k):
        k = jnp.concatenate([_zip(k[0:56], k[56:112]), jnp.zeros((8, 128), I32)], axis=0)
        k = pltpu.bitcast(_bf(k).T, I32)
        for i, keys in enumerate(_unzip(k)):
            kn[g, i, pl.ds(c * 32, 32)] = _words(keys)

    def b_q(c, g, q):
        lo = _iota((8, 128), 0) < 4
        r1 = pltpu.roll(q[24:56], 32, 1)
        r2 = pltpu.roll(q[56:88], 64, 1)
        r3 = pltpu.roll(q[80:112], 96, 1)
        qr[c, g] = _zip(
            jnp.concatenate(
                [q[0:24], jnp.where(lo, q[24:32], r1[0:8]), r1[8:32]], axis=0),
            jnp.concatenate(
                [r2[0:24], jnp.where(lo, r2[24:32], r3[0:8]), r3[8:32]], axis=0))

    def b_v(c, g, v):
        lo = _iota((8, 128), 0) < 4
        for e in range(2):
            ve = v[56 * e:56 * e + 56]
            vp[c, 4 * g + 2 * e] = _words(jnp.concatenate(
                [ve[0:24], jnp.where(lo, ve[24:32], 1.0)], axis=0))
            vp[c, 4 * g + 2 * e + 1] = _words(jnp.concatenate(
                [jnp.where(lo, 1.0, ve[24:32]), ve[32:56]], axis=0))

    def scores(blk, g):
        q = qr[blk, g]
        out = [None] * 4
        gate = next_round()
        for t in (3, 2, 1, 0) if g % 2 else (0, 1, 2, 3):
            qt = _bf(jnp.concatenate(
                [q & qmask[t, 0:56], jnp.zeros((8, 128), I32)], axis=0))
            end = blk * 128 + 32 * t + 32
            start = max(end - 288, 0)
            keys = [kn[g, i, start // 4:end // 4] for i in range(2)]
            keys = jnp.concatenate(keys, axis=0)
            out[t] = _dot(gate(keys), qt)
        if g == 0 and blk in ALIGN:
            spread(out, 128)
        return out

    def b_qk(c, g):
        key, qry = 2 * _iota((16, 128), 0), _iota((16, 128), 1) & 31
        for t, s in enumerate(scores(c, g)):
            n = s.shape[0] // 2
            halves = []
            for i in range(2):
                h = s[i * n:i * n + n]
                edge = jnp.where(key + i <= qry, h[n - 16:],
                                 h[0:16] if n == 144 else -1e9 * LOG2E)
                halves.append(jnp.concatenate(
                    [h[max(n - 128, 0):n - 16], edge], axis=0) if n > 16 else edge)
            m = jnp.max(jnp.concatenate(halves, axis=0), axis=0, keepdims=True)
            live["s", g, t] = (halves, m)

    def b_exp(t):
        def stage(c, g):
            halves, m = live.pop(("s", g, t))
            pbuf[g, t, 128 - halves[0].shape[0]:] = _zip(
                *[jnp.exp2(h - m) for h in halves])
        return stage

    def b_pv(i):
        def pick(cond, a, b):
            if a is None and b is None:
                return None
            return jnp.where(cond, 0 if a is None else a, 0 if b is None else b)

        def stage(c, g):
            if c - 2 + i < 0:
                return
            ln = _iota((16, 128), 1)
            odd, upper = (ln & 32) != 0, (ln & 64) != 0
            heads = [[] for _ in range(4)]
            for u in range(4):
                pc = []
                for t in range(4):
                    k = 4 * i + u - t
                    if k in (0, 8):
                        pc.append(pbuf[g, t, 112:128] & pmask[k // 8])
                    else:
                        pc.append(pbuf[g, t, 16 * k - 16:16 * k] if 0 < k < 8 else None)
                y = [pick(odd, pc[(k + 1) % 4], pc[k]) for k in range(4)]
                for j in range(4):
                    heads[j].append(pick(upper, y[(2 - j) % 4], y[(-j) % 4]))
            acc = live.get(("o", c, g))
            res = [_dot(_bf(vp[c - 2 + i, 4 * g + j]),
                        _bf(jnp.concatenate(heads[j], axis=0))) for j in range(4)]
            live["o", c, g] = res if acc is None else [a + o for a, o in zip(acc, res)]
        return stage

    def b_fin(c, g):
        res = [o if j == 0 else pltpu.roll(o, 128 - 32 * j, 1)
               for j, o in enumerate(live.pop(("o", c, g)))]
        lo = _iota((8, 128), 0) < 4
        outs = []
        for e in range(2):
            u, w = res[2 * e], res[2 * e + 1]
            num = jnp.concatenate(
                [u[0:24], jnp.where(lo, u[24:32], w[0:8]), w[8:32]], axis=0)
            den = pltpu.roll(jnp.where(lo, w[0:8], u[24:32]), 4, 0)
            outs.append(_pair_scale(num, den))
        att[1, c % 4, pl.ds(56 * g, 56)] = _zip(*outs)

    def b_out(c, g, y):
        rows = pl.ds(112 * g, 112)
        xio[rows, 128 * c:128 * c + 128] = (xt[c, rows] + y).astype(BF16)
        if g == 3 and c + 1 in OUT_CUTS:
            o_copies[OUT_CUTS.index(c + 1) - 1].start()

    def load_x(c, g):
        if g == 0:
            if c in IN_CUTS[2:]:
                for cp in [x_copies[2]] + w_copies[2:4]:
                    cp.wait()
                for cp in w_copies[4:]:
                    cp.start()
            xt[c] = xio[:, 128 * c:128 * c + 128].astype(F32)

    def transpose(w, src, i):
        n = min(128, src.shape[1] - i)
        rows = pl.ds((w * D + i) // 2, n // 2)
        a = src[:, i:i + n].astype(F32)
        for kh in range(2):
            j = kh * HD
            wt[kh, rows] = _words(_bf(_zip(a[j:j + 112], a[j + 112:j + HD])).T)

    def transpose_out(w, src, i):
        n = min(128, D - i)
        a = src[:, i:i + n].astype(F32)
        a = [_zip(a[j:j + 56], a[j + 56:j + 112]) for j in range(0, D, 112)]
        wo[w, i // 2:(i + n) // 2] = _words(_bf(jnp.concatenate(a, axis=0)).T)

    def factors(w, h, cols):
        quad = []
        for g in (2 * h, 2 * h + 1):
            for kh in range(2):
                a = wt[kh, pl.ds(w * HD + 56 * g, 56), cols]
                if w in (AQ, AK):
                    a = _dot(bdt[g], _bf(a)) * LOG2E
                    quad.append((a[0:56], a[56:112]))
                elif w == BQ:
                    quad.append([x * (DH ** -0.5 * LOG2E) for x in _unzip(a)])
                else:
                    quad.append(_unzip(a))
        even, odd = [_strassen_left(*[a[i] for a in quad]) for i in range(2)]
        for r in range(7):
            ws[w, r, pl.ds(56 * h, 56), cols] = pin(_zip(even[r], odd[r]), PREP_DUE)

    def weight_steps(w, src, lo, hi, parts):
        return ([(transpose, w, src, i) for i in range(lo, hi, 128)]
                + [(factors, p, h, cols) for p in parts
                   for h in range(2) for cols in (pl.ds(0, 128), pl.ds(128, HD - 128))])

    late = (weight_steps(AQ, rawa, 0, 384, [AQ]) + [(transpose_out, 0, rawoa, i) for i in range(0, D, 128)]
            + [(lambda: None,)] * 4 + [(lambda: [cp.wait() for cp in w_copies[4:]],)]
            + weight_steps(BQ, rawb, 0, 3 * D, [BK, BQ, BV])
            + [(transpose_out, 1, rawob, i) for i in range(0, D, 128)])

    def prep(c, g):
        for step in late[4 * c + g:4 * c + g + 1]:
            step[0](*step[1:])

    x_copies[0].wait()
    for c in range(2):
        load_x(c, 0)
    for stage in (stats(xna), norm(xna)):
        for g in range(4):
            stage(0, g)
    w_copies[0].wait()
    load_phi()
    for cp in [x_copies[2]] + w_copies[2:4]:
        cp.start()
    for step in weight_steps(AQ, rawa, 896, 3 * D, [AV]):
        step[0](*step[1:])
    w_copies[1].wait()
    for vals in due:
        vals.clear()
    steps = weight_steps(AQ, rawa, 384, 896, [AK])
    for u in range(8):
        proj(AV, a_v)(*divmod(u, 4))
        for step in steps[2 * u:2 * u + 2]:
            step[0](*step[1:])
    x_copies[1].wait()
    load_x(2, 0)

    U = 4 * NB
    plan = [(load_x, -12), (prep, 4 * IN_CUTS[2] - 12), (stats(xna), -8),
            (norm(xna), -4), (proj(AK, lambda *a: a_k(*a, first=True)), 0),
            (lambda c, g: c < 2 or proj(AV, a_v)(c, g), 1), (a_kv, 5)]
    t0 = U + 4
    for last in (False, True):
        gap, order = GAP[last], ORDER[last]
        t0 += gap[6]
        t1 = t0 + 5 + gap[0]
        t2 = t1 + 15 + gap[1]
        t3 = t2 + 6 + gap[2]
        t4 = t3 + 2 + gap[3]
        t5 = t4 + 5 + gap[4]
        t6 = t5 + 15 + gap[5]
        stages = {
            "S": [(b_qk, t3)], "N": [(a_num, t0)],
            "O": [(out_proj(0, residual), t1)],
            "W": [(out_proj(1, b_out if last else residual), t5)],
            "F": [(proj(AQ, a_q), t0 - 4 - gap[7])],
            "K": [(proj(BK, b_k), t2 + gap[8])], "Q": [(proj(BQ, b_q), t2 + gap[9])],
            "V": [(proj(BV, b_v), t2 + gap[10])],
            "l": [(stats(xnb), t1 + 6 + min(gap[11], gap[1]))], "n": [(norm(xnb), t2 - 5)],
            "e": [(b_exp(t), t3 + 1) for t in range(4)],
            "0": [(b_pv(0), t4)], "1": [(b_pv(1), t4)], "2": [(b_pv(2), t4)],
            "G": [(proj(AK, a_k), t6)], "H": [(proj(AV, a_v), t6 + 1)],
            "m": [(stats(xna), t5 + 6 + min(gap[12], gap[5]))], "o": [(norm(xna), t6 - 5)],
            "Z": [(a_kv, t6 + 5)]}
        for name in order:
            plan += stages[name]
        plan.append((b_fin, t4))
        t0 = t6 + U + 4
    for u in range(max(t for _, t in plan) + U):
        if u in RESET:
            live["spread"] = True
        for stage, t in plan:
            if 0 <= u - t < U:
                stage(*divmod(u - t, 4))

    for cp in o_copies:
        cp.wait()


@jax.jit
def pallas_interleave_layers__linear_kernel_hedgehog__sliding_block__prompt_kernel(
    A_x: jax.Array,
    A_wqkv: jax.Array,
    A_w_phi: jax.Array,
    A_wo: jax.Array,
    B_x: jax.Array,
    B_wqkv: jax.Array,
    B_wo: jax.Array,
):
    del B_x
    hbm = pl.BlockSpec(memory_space=pltpu.MemorySpace.HBM)
    out = pl.pallas_call(
        _kernel,
        out_shape=jax.ShapeDtypeStruct((D, S), A_x.dtype),
        in_specs=[hbm] * 6,
        out_specs=hbm,
        scratch_shapes=[
            pltpu.VMEM((D, S), BF16),
            pltpu.VMEM((D, 3 * D), BF16),
            pltpu.VMEM((D, 3 * D), BF16),
            pltpu.VMEM((D, D), BF16),
            pltpu.VMEM((D, D), BF16),
            pltpu.VMEM((D, DH), BF16),
            pltpu.VMEM((D + H, 128), F32),
            pltpu.VMEM((4, 128, 128), F32),
            pltpu.VMEM((2, HD, D), I32),
            pltpu.VMEM((2, 6 * HD, HD), I32),
            pltpu.VMEM((6, 7, HD // 2, HD), I32),
            pltpu.VMEM((2, NB // 2, 7, HD // 2, 128), I32),
            pltpu.VMEM((6, 2, 4, 112, 128), F32),
            pltpu.VMEM((4, 8, 56, 128), I32),
            pltpu.VMEM((4, 8, 32, 128), I32),
            pltpu.VMEM((NB, 8, 56, 128), I32),
            pltpu.VMEM((2, 4, HD, 128), I32),
            pltpu.VMEM((4, 4, 128, 128), I32),
            pltpu.VMEM((NB, D, 128), F32),
            pltpu.VMEM((8, 64, 112), F32),
            pltpu.VMEM((8, 32, 112), I32),
            pltpu.VMEM((NB, 4, 56, 128), I32),
            pltpu.VMEM((4, 2, S // 4, 128), I32),
            pltpu.VMEM((NB, H, 16, 128), I32),
            pltpu.VMEM((4, 64, 128), I32),
            pltpu.VMEM((2, 16, 128), I32),
            pltpu.VMEM((8, 128), I32),
            pltpu.SemaphoreType.DMA((7,)),
            pltpu.SemaphoreType.DMA((len(IN_CUTS) - 1,)),
            pltpu.SemaphoreType.DMA((len(OUT_CUTS) - 1,)),
        ],
        compiler_params=pltpu.CompilerParams(vmem_limit_bytes=96 * 1024 * 1024),
    )(A_x.reshape(S, D).T, A_wqkv, A_w_phi.transpose(1, 0, 2).reshape(D, DH),
      A_wo, B_wqkv, B_wo)
    return out.T.reshape(A_x.shape)
```
